```python
import os as _os
_os.environ.setdefault("JAX_PLATFORMS", "cpu")
import jax
import jax.numpy as jnp

def _softmax(x, axis=-1):
    return jax.nn.softmax(x, axis=axis)
def _gelu(x):
    return jax.nn.gelu(x, approximate=True)
def _silu(x):
    return jax.nn.silu(x)
def _sigmoid(x):
    return jax.nn.sigmoid(x)
def _layernorm(x, axis=-1, eps=1e-5):
    m = jnp.mean(x, axis=axis, keepdims=True)
    v = jnp.var(x, axis=axis, keepdims=True)
    return (x - m) / jnp.sqrt(v + eps)
def _scatter_add(tgt, idx, src, axis=0):
    return tgt.at[idx].add(src)
def _segment_sum(src, seg, n):
    return jax.ops.segment_sum(src, seg, n)
class _Rng:
    def __init__(self, key):
        self._k = key
    def _next(self):
        self._k, sub = jax.random.split(self._k)
        return sub
    def normal(self, shape):
        return jax.random.normal(self._next(), shape, dtype=jnp.bfloat16)
    def randint(self, lo, hi, shape):
        return jax.random.randint(self._next(), shape, lo, hi, dtype=jnp.int32)
    def uniform(self, shape, lo=0.0, hi=1.0):
        return jax.random.uniform(self._next(), shape, jnp.bfloat16, lo, hi)
    def permutation(self, n):
        return jax.random.permutation(self._next(), n)


kernel_name = 'gated_mix__sliding_local_dilated__moe_arch_mod__prompt'

def setup_inputs():
    _rng = _Rng(jax.random.key(int.from_bytes(__import__("os").urandom(4), "little")))
    _w = (lambda a: (lambda t: t.astype(jnp.bfloat16) if jnp.issubdtype(t.dtype, jnp.floating) else t)(jnp.asarray(a)))
    def _A_setup():
        B, S, D = 1, 2048, 640
        return {
            "x": _w((lambda *s: _rng.normal(s) * 0.05)(B, S, D)),
            "wqkv": _w((lambda *s: _rng.normal(s) * 0.8)(D, 3 * D)),
            "wo": _w((lambda *s: _rng.normal(s) * 0.05)(D, D)),
        }
    _A_in = _A_setup()

    def _B_setup():
        B, S, D, F, C = 1, 2048, 640, 1728, 1
        return {
            "x": _w((lambda *s: _rng.normal(s) * 0.05)(B, S, D)),
            "w_r": _w((lambda *s: _rng.normal(s) * 1.6)(D)),
            "w_gate": _w((lambda *s: _rng.normal(s) * 0.4)(D, F)),
            "w_up": _w((lambda *s: _rng.normal(s) * 0.4)(D, F)),
            "w_down": _w((lambda *s: _rng.normal(s) * 0.4)(F, D)),
        }
    _B_in = _B_setup()

    return {
        "A_x": _A_in["x"],
        "A_wqkv": _A_in["wqkv"],
        "A_wo": _A_in["wo"],
        "B_x": _B_in["x"],
        "B_w_r": _B_in["w_r"],
        "B_w_gate": _B_in["w_gate"],
        "B_w_up": _B_in["w_up"],
        "B_w_down": _B_in["w_down"],
        "gate_w": _w((lambda *s: _rng.normal(s) * 0.05)(640) * 16.0),
    }

def reference(A_x, A_wqkv, A_wo, B_x, B_w_r, B_w_gate, B_w_up, B_w_down, gate_w):
    def _A_ref(x, wqkv, wo):
        B, S, D = x.shape
        H = 32; Dh = D // H
        W, dil = 8, 2
        qkv = (lambda x, *d: x.transpose(*d))((x @ wqkv).reshape(B, S, 3, H, Dh), 2, 0, 3, 1, 4)
        q, k, v = qkv[0], qkv[1], qkv[2]
        scale = Dh ** -0.5
        pos = jnp.arange(S)
        off = jnp.arange(W) * dil
        idx = pos[:, None] - off[None, :]
        mask = idx >= 0
        idx_c = jnp.where(mask, idx, 0).reshape(-1)
        kg = k[:, :, idx_c, :].reshape(B, H, S, W, Dh)
        vg = v[:, :, idx_c, :].reshape(B, H, S, W, Dh)
        logits = jnp.einsum("bhsd,bhswd->bhsw", q, kg) * scale
        logits = jnp.where(mask[None, None, :, :], logits, -1e9)
        attn = _softmax(logits, axis=-1)
        o = jnp.einsum("bhsw,bhswd->bhsd", attn, vg)
        return (lambda x, *d: x.transpose(*d))(o, 0, 2, 1, 3).reshape(B, S, D) @ wo

    def _B_ref(x, w_r, w_gate, w_up, w_down):
        B, S, D = x.shape
        C = 1
        r = x @ w_r
        idx = jnp.argsort(-r, axis=-1)[:, :C]
        idx_e = jnp.repeat(idx.reshape(B, C, 1), D, axis=2)
        x_sel = jnp.take_along_axis(x, idx_e, axis=1)
        g = _silu(x_sel @ w_gate)
        u = x_sel @ w_up
        y = (g * u) @ w_down
        r_sel = _sigmoid(jnp.take_along_axis(r, idx, axis=1))
        y = y * r_sel.reshape(B, C, 1)
        b_off = (jnp.arange(B) * S).reshape(B, 1)
        flat_idx = (idx + b_off).reshape(B * C)
        zero = (x * 0.0).reshape(B * S, D)
        upd = _scatter_add(zero, flat_idx, y.reshape(B * C, D), axis=0)
        return x + upd.reshape(B, S, D)

    x = A_x
    g = _sigmoid((x * gate_w).sum(-1, keepdims=True))
    a = _A_ref(x, A_wqkv, A_wo)
    b = _B_ref(x, B_w_r, B_w_gate, B_w_up, B_w_down)
    return g * a + (1 - g) * b
```

```python
import functools

import jax
import jax.numpy as jnp
from jax import lax
from jax.experimental import pallas as pl
from jax.experimental.pallas import tpu as pltpu

S, D, H, DH, W, DIL, F = 2048, 640, 32, 20, 8, 2, 1728
NC = D // 128
HALO = 16
SCALE = DH ** -0.5
LOG2E = 1.4426950408889634

WB = S
FB = S + 4 * D
PAD = FB + 3 * F

T = 64
RB = 16
P0 = 256
XC = (0, 256, 640, 2048)
OC = (0, 768, 1536, 1792, 1920, 2048)
W_GROUPS = ((0, 1, 3, 5), (0, 3, 5), (0, 3, 5))
DMA_AHEAD = 4
GATE_RATE = (1.5, 2.25)
ATTN_RATE = 1.75
OUT_RATE = 1.75
OUT_DELAY = 2
OUT_RESERVE = 64
FFN_FROM = 960
FFN_RATE = 288
DEP_DELAY = 3

f32, bf16, u32 = jnp.float32, jnp.bfloat16, jnp.uint32
NT = (((1,), (1,)), ((), ()))


def _pk(x):
    return pltpu.bitcast(x.astype(bf16), u32)


def _upk(x):
    return pltpu.bitcast(x, bf16)


def _sigmoid(z):
    return 0.5 * jnp.tanh(0.5 * z) + 0.5


def _kernel(x_hbm, wqkv_hbm, wo_hbm, wr_hbm, wg_hbm, wu_hbm, wd_hbm, gw_hbm, out_hbm,
            wr_ref, gw_ref, x_v, out_v, tmp, wt, wop, xp, g_s, q_s, k_s, v_s, o_s,
            xsem, wsem, fsem, osem):
    def xcopy(i):
        sl = pl.ds(XC[i], XC[i + 1] - XC[i])
        return pltpu.make_async_copy(x_hbm.at[sl], x_v.at[sl], xsem.at[i])

    def wcopy(p, k0, k1):
        n = (k1 - k0) * 128
        return pltpu.make_async_copy(
            wqkv_hbm.at[pl.ds(k0 * 128, n), pl.ds(p * D, D)],
            x_v.at[pl.ds(WB + p * D + k0 * 128, n)], wsem.at[p * NC + k0])

    def ocopy(i):
        sl = pl.ds(OC[i], OC[i + 1] - OC[i])
        return pltpu.make_async_copy(out_v.at[sl], out_hbm.at[sl], osem.at[i])

    wocopy = pltpu.make_async_copy(wo_hbm, x_v.at[pl.ds(WB + 3 * D, D)], wsem.at[15])
    fcopies = [pltpu.make_async_copy(a, x_v.at[pl.ds(FB + j * F, F)], fsem.at[j])
               for j, a in enumerate((wg_hbm, wu_hbm, wd_hbm))]
    vcopies = [pltpu.make_async_copy(gw_hbm, gw_ref, wsem.at[16]),
               pltpu.make_async_copy(wr_hbm, wr_ref, wsem.at[17])]

    def pin(v):
        x_v[PAD:PAD + 16, 0:128] = v

    def prep_w(p, kt):
        r0 = WB + p * D + kt * 128
        for nt in range(NC):
            t = x_v[r0:r0 + 128, nt * 128:(nt + 1) * 128].astype(f32)
            tmp[kt, nt * 128:(nt + 1) * 128, :] = t.T
        for d in range(DH):
            rows = tmp[kt, pl.ds(d, H, stride=DH), :]
            wt[kt, (p * D + d * H) // 2:(p * D + (d + 1) * H) // 2, :] = _pk(rows)

    def prep_wo():
        for kt in range(NC):
            tmp[kt] = x_v[WB + 3 * D:WB + 4 * D, kt * 128:(kt + 1) * 128].astype(f32)
        for kt in range(NC):
            for d in range(DH):
                rows = tmp[kt, pl.ds(d, H, stride=DH), :]
                wop[kt, d * H // 2:(d + 1) * H // 2, :] = _pk(rows)

    dsts = (q_s, k_s, v_s)

    def rows_of(ref, s0, t):
        return jnp.concatenate([_upk(ref[kt, s0 // 2:(s0 + t) // 2, :]) for kt in range(NC)], axis=1)

    def xpack(s0, t):
        for c in range(NC):
            xp[c, s0 // 2:(s0 + t) // 2, :] = pltpu.bitcast(x_v[s0:s0 + t, c * 128:(c + 1) * 128], u32)

    def partial_proj(p, kt):
        xl = _upk(xp[kt, 0:P0 // 2, :])
        for c in range(NC):
            n0 = p * D + c * 128
            r = lax.dot_general(xl, _upk(wt[kt, n0 // 2:n0 // 2 + 64, :]), NT, preferred_element_type=f32)
            if kt > 0:
                r = r + dsts[p][c, HALO:HALO + P0, :]
            dsts[p][c, HALO:HALO + P0, :] = r
            if kt == NC - 1 and p > 0:
                dsts[p][c, 0:HALO, :] = jnp.broadcast_to(r[0:1], (HALO, 128))
            if c == 0:
                v = r[P0 - 16:P0].astype(bf16)
        return v

    def proj(s0, t, p):
        for c in range(NC):
            r = lax.dot_general(rows_of(xp, s0, t), rows_of(wt, p * D + c * 128, 128), NT,
                                preferred_element_type=f32)
            dsts[p][c, HALO + s0:HALO + s0 + t, :] = r
            v = r[t - 16:t].astype(bf16)
        return v

    def attn(s0):
        q = [q_s[c, HALO + s0:HALO + s0 + RB, :] for c in range(NC)]
        ls = []
        for w in range(W):
            b = HALO + s0 - DIL * w
            p_ = q[0] * k_s[0, b:b + RB, :]
            for c in range(1, NC):
                p_ = p_ + q[c] * k_s[c, b:b + RB, :]
            p_ = p_ + pltpu.roll(p_, 64, 1)
            p_ = p_ + pltpu.roll(p_, 32, 1)
            if s0 < DIL * w:
                row = lax.broadcasted_iota(jnp.int32, (RB, 128), 0) + s0
                p_ = jnp.where(row >= DIL * w, p_, -1e9 / SCALE)
            ls.append(p_)
        m = functools.reduce(jnp.maximum, ls)
        es = [jnp.exp2((l - m) * (SCALE * LOG2E)) for l in ls]
        ssum = functools.reduce(jnp.add, es)
        inv = pl.reciprocal(ssum, approx=True)
        inv = inv * (2.0 - ssum * inv)
        for c in range(NC):
            acc = es[0] * v_s[c, HALO + s0:HALO + s0 + RB, :]
            for w in range(1, W):
                b = HALO + s0 - DIL * w
                acc = acc + es[w] * v_s[c, b:b + RB, :]
            o_s[c, s0 // 2:(s0 + RB) // 2, :] = _pk(acc * inv)

    def outp(s0, t, c):
        a = jnp.dot(rows_of(o_s, s0, t), _upk(wop[c]), preferred_element_type=f32)
        xf = x_v[s0:s0 + t, c * 128:(c + 1) * 128].astype(f32)
        g = g_s[s0:s0 + t, :]
        out_v[s0:s0 + t, c * 128:(c + 1) * 128] = (xf + g * (a - xf)).astype(bf16)

    def gate_and_route(s0, t, best):
        xf = x_v[s0:s0 + t, :].astype(f32)
        g_s[s0:s0 + t, :] = _sigmoid(jnp.broadcast_to(jnp.sum(xf * gw, axis=1, keepdims=True), (t, 128)))
        r = jnp.broadcast_to(jnp.sum(xf * wr, axis=1, keepdims=True), (t, 128)).astype(bf16).astype(f32)
        row = lax.broadcasted_iota(jnp.int32, (8, 128), 0)
        for j in range(t // 8):
            rj = r[j * 8:(j + 1) * 8]
            ij = row + (s0 + j * 8)
            if best is None:
                best = (rj, ij)
            else:
                upd = rj > best[0]
                best = (jnp.where(upd, rj, best[0]), jnp.where(upd, ij, best[1]))
        return best

    def ffn_select(best):
        bv, bi = best
        mx = jnp.max(bv, axis=0, keepdims=True)
        idx = jnp.min(jnp.where(bv == mx, bi, S - 1)[:, 0:1])
        base = pl.multiple_of((idx // 16) * 16, 16)
        sel = lax.broadcasted_iota(jnp.int32, (16, D), 0) == (idx - base)
        xrows = x_v[pl.ds(base, 16), :].astype(f32)
        xs = jnp.sum(jnp.where(sel, xrows, 0.0), axis=0, keepdims=True)
        return idx, base, sel, xs, mx

    def ffn_part(st, n0, n1, yacc):
        x8 = jnp.broadcast_to(st[3], (8, D))
        for n in range(n0, n1, 8):
            gg = jnp.sum(x_v[FB + n:FB + n + 8, :].astype(f32) * x8, axis=1, keepdims=True)
            uu = jnp.sum(x_v[FB + F + n:FB + F + n + 8, :].astype(f32) * x8, axis=1, keepdims=True)
            hh = gg * _sigmoid(gg) * uu
            t_ = hh * x_v[FB + 2 * F + n:FB + 2 * F + n + 8, :].astype(f32)
            yacc = t_ if yacc is None else yacc + t_
        return yacc

    def ffn_scatter(st, yacc, frontier):
        idx, base, sel, xs, mx = st
        y = jnp.sum(yacc, axis=0, keepdims=True) * _sigmoid(mx[:, 0:1])
        gsel = _sigmoid(jnp.sum(xs * gw, axis=1, keepdims=True))
        xrows = x_v[pl.ds(base, 16), :].astype(f32)
        x_v[pl.ds(base, 16), :] = jnp.where(sel, xrows + y, xrows).astype(bf16)
        base1 = pl.multiple_of(jnp.minimum(base, frontier - 16), 16)
        sel1 = lax.broadcasted_iota(jnp.int32, (16, D), 0) == (idx - base1)
        orows = out_v[pl.ds(base1, 16), :].astype(f32)
        out_v[pl.ds(base1, 16), :] = jnp.where(sel1, orows + (1.0 - gsel) * y, orows).astype(bf16)
        return jnp.broadcast_to(y[:, :128], (8, 128))

    order = (1, 2, 0)
    pieces = [(p, kt) for p in order for kt in range(NC)]
    wcs = {}
    for j, p in enumerate(order):
        for k0, k1 in zip(W_GROUPS[j][:-1], W_GROUPS[j][1:]):
            wcs[j * NC + k0] = wcopy(p, k0, k1)
    queue = list(wcs.values()) + [xcopy(1), wocopy, xcopy(2)] + fcopies
    xcopy(0).start()
    for c in queue[:DMA_AHEAD]:
        c.start()
    qi = DMA_AHEAD
    xcopy(0).wait()
    xpack(0, P0)
    vals = []
    for i, (p, kt) in enumerate(pieces):
        if i in wcs:
            if i >= 2:
                pin(vals[i - 2])
            wcs[i].wait()
            if qi < len(queue):
                queue[qi].start()
                qi += 1
        if i == 4:
            for c in vcopies:
                c.start()
        prep_w(p, kt)
        vals.append(partial_proj(p, kt))
    pin(vals[13])
    xcopy(1).wait()
    while qi < len(queue):
        queue[qi].start()
        qi += 1
    for c in vcopies:
        c.wait()
    xpack(P0, T)
    gw = gw_ref[...].astype(f32).reshape(1, D)
    wr = wr_ref[...].astype(f32).reshape(1, D)

    zero = jnp.minimum(jnp.max(pltpu.bitcast(xp[0, 0:8, :], jnp.int32) & 0xFFFF), 0)
    zero = pl.multiple_of(zero, 16)

    best = st = yacc = odep = None
    lastv = vals[14]
    a_pos, b_pos, c_pos = P0, 0, 0
    x_pos, packed, f_pos = 0, P0 + T, 0
    xacc = bacc = cacc = 0.0
    xi, oi = 2, 0
    ffn_ready = fixed = False
    delayed = []
    while c_pos < S:
        if a_pos == P0 + T:
            pin(lastv)
            wocopy.wait()
            prep_wo()
            pin(lastv)
        if xi == 2 and a_pos + T >= XC[2]:
            pin(lastv)
            xcopy(2).wait()
            xi = 3
        od, odep, dep = odep, None, None
        if x_pos < S:
            xacc = min(xacc + GATE_RATE[xi - 2] * T, XC[xi])
            tgt = min(XC[xi], int(xacc) // 16 * 16)
            if tgt > x_pos:
                best = gate_and_route(x_pos, tgt - x_pos, best)
                x_pos = tgt
                dep = best[0]
        elif st is None:
            st = ffn_select(best)
            dep = jnp.broadcast_to(st[3][:, :128], (8, 128))
        elif not ffn_ready and a_pos >= FFN_FROM:
            pin(lastv)
            for c in fcopies:
                c.wait()
            ffn_ready = True
        if ffn_ready and f_pos < F:
            f1 = min(F, f_pos + FFN_RATE)
            yacc = ffn_part(st, f_pos, f1, yacc)
            f_pos = f1
            dep = functools.reduce(jnp.add, [yacc[:, c * 128:(c + 1) * 128] for c in range(NC)])
        elif ffn_ready and not fixed:
            assert packed == S and c_pos >= 16
            dep = ffn_scatter(st, yacc, c_pos)
            fixed = True
        delayed.append(dep)
        dep = delayed.pop(0) if len(delayed) > DEP_DELAY else None
        if od is not None:
            dep = od if dep is None else pltpu.bitcast(dep, u32) | pltpu.bitcast(od, u32)
        if c_pos > 0:
            md = pltpu.bitcast(out_v[pl.ds(zero, 16), 0:128], u32)
            dep = md if dep is None else md | pltpu.bitcast(dep, u32)
        tgt = min(XC[xi], max(x_pos, a_pos + 2 * T))
        if tgt > packed:
            xpack(packed, tgt - packed)
            packed = tgt
        nxt = a_pos + T
        if dep is not None and nxt < S:
            assert nxt + 16 <= packed
            sl = slice(nxt // 2, nxt // 2 + 8)
            xp[0, sl, :] = jnp.where(best[1] < 0, pltpu.bitcast(dep, u32), xp[0, sl, :])
        if a_pos < S:
            for p in (order if a_pos + T < S else (0, 1, 2)):
                lastv = proj(a_pos, T, p)
        bacc = min(bacc + ATTN_RATE * T, a_pos)
        nb = max(0, int(bacc) // RB * RB - b_pos)
        reserve = OUT_RESERVE if (a_pos < S and a_pos + 4 * T >= S) else 0
        cacc = min(cacc + OUT_RATE * T, b_pos - reserve)
        if a_pos < P0 + OUT_DELAY * T:
            cacc = 0.0
        nc = max(0, int(cacc) // 16 * 16 - c_pos)
        if nc:
            assert c_pos + nc <= min(x_pos, b_pos)
            for c in range(NC):
                outp(c_pos, nc, c)
        for s in range(b_pos, b_pos + nb, RB):
            attn(s)
        a_pos = min(S, a_pos + T)
        b_pos += nb
        c_pos += nc
        while fixed and oi < len(OC) - 1 and OC[oi + 1] <= c_pos:
            ocopy(oi).start()
            oi += 1
            if a_pos < S:
                dyn = pl.multiple_of(S + 16 * (st[0] >> 12), 16)
                out_v[pl.ds(dyn, 16), 0:128] = jnp.zeros((16, 128), bf16)
                odep = out_v[pl.ds(dyn, 16), 0:128]
    assert oi == len(OC) - 1
    for i in range(len(OC) - 1):
        ocopy(i).wait()


@jax.jit
def pallas_gated_mix__sliding_local_dilated__moe_arch_mod__prompt_kernel(
    A_x: jax.Array,
    A_wqkv: jax.Array,
    A_wo: jax.Array,
    B_x: jax.Array,
    B_w_r: jax.Array,
    B_w_gate: jax.Array,
    B_w_up: jax.Array,
    B_w_down: jax.Array,
    gate_w: jax.Array,
):
    del B_x
    hbm = pl.BlockSpec(memory_space=pltpu.HBM)
    out = pl.pallas_call(
        _kernel,
        out_shape=jax.ShapeDtypeStruct((S, D), bf16),
        in_specs=[hbm] * 8,
        out_specs=hbm,
        scratch_shapes=[
            pltpu.VMEM((D,), bf16),
            pltpu.VMEM((D,), bf16),
            pltpu.VMEM((PAD + 16, D), bf16),
            pltpu.VMEM((S + 32, D), bf16),
            pltpu.VMEM((NC, D, 128), f32),
            pltpu.VMEM((NC, 3 * D // 2, 128), u32),
            pltpu.VMEM((NC, D // 2, 128), u32),
            pltpu.VMEM((NC, S // 2, 128), u32),
            pltpu.VMEM((S, 128), f32),
            pltpu.VMEM((NC, S + HALO, 128), f32),
            pltpu.VMEM((NC, S + HALO, 128), f32),
            pltpu.VMEM((NC, S + HALO, 128), f32),
            pltpu.VMEM((NC, S // 2, 128), u32),
            pltpu.SemaphoreType.DMA((len(XC) - 1,)),
            pltpu.SemaphoreType.DMA((18,)),
            pltpu.SemaphoreType.DMA((3,)),
            pltpu.SemaphoreType.DMA((len(OC) - 1,)),
        ],
        compiler_params=pltpu.CompilerParams(
            vmem_limit_bytes=100 * 1024 * 1024,
            flags={"XLA_TPU_RESCHEDULE_DMA_DONES": True},
        ),
        name="gmix",
    )(A_x.reshape(S, D), A_wqkv, A_wo, B_w_r, B_w_gate.T, B_w_up.T, B_w_down, gate_w)
    return out.reshape(1, S, D)
```
